```python
import os as _os
_os.environ.setdefault("JAX_PLATFORMS", "cpu")
import jax
import jax.numpy as jnp

def _softmax(x, axis=-1):
    return jax.nn.softmax(x, axis=axis)
def _gelu(x):
    return jax.nn.gelu(x, approximate=True)
def _silu(x):
    return jax.nn.silu(x)
def _sigmoid(x):
    return jax.nn.sigmoid(x)
def _layernorm(x, axis=-1, eps=1e-5):
    m = jnp.mean(x, axis=axis, keepdims=True)
    v = jnp.var(x, axis=axis, keepdims=True)
    return (x - m) / jnp.sqrt(v + eps)
def _scatter_add(tgt, idx, src, axis=0):
    return tgt.at[idx].add(src)
def _segment_sum(src, seg, n):
    return jax.ops.segment_sum(src, seg, n)
class _Rng:
    def __init__(self, key):
        self._k = key
    def _next(self):
        self._k, sub = jax.random.split(self._k)
        return sub
    def normal(self, shape):
        return jax.random.normal(self._next(), shape, dtype=jnp.bfloat16)
    def randint(self, lo, hi, shape):
        return jax.random.randint(self._next(), shape, lo, hi, dtype=jnp.int32)
    def uniform(self, shape, lo=0.0, hi=1.0):
        return jax.random.uniform(self._next(), shape, jnp.bfloat16, lo, hi)
    def permutation(self, n):
        return jax.random.permutation(self._next(), n)


kernel_name = 'concat_heads__spectral_gfnet__mha_block__prompt'

def setup_inputs():
    _rng = _Rng(jax.random.key(int.from_bytes(__import__("os").urandom(4), "little")))
    _w = (lambda a: (lambda t: t.astype(jnp.bfloat16) if jnp.issubdtype(t.dtype, jnp.floating) else t)(jnp.asarray(a)))
    def _A_setup():
        B, S, D = 1, 2048, 576
        Df = D // 2 + 1
        return {
            "x": _w((lambda *s: _rng.normal(s) * 0.05)(B, S, D)),
            "w_r": _w((lambda *s: _rng.normal(s) * 0.05)(S, Df) * 0.02),
            "w_i": _w((lambda *s: _rng.normal(s) * 0.05)(S, Df) * 0.02),
        }
    _A_in = _A_setup()

    def _B_setup():
        B, S, D, H = 1, 2048, 576, 32
        return {
            "x": _w((lambda *s: _rng.normal(s) * 0.1)(B, S, D)),
            "wqkv": _w((lambda *s: _rng.normal(s) * 0.1)(D, 3 * D)),
            "wo": _w((lambda *s: _rng.normal(s) * 0.05)(D, D)),
        }
    _B_in = _B_setup()

    return {
        "A_x": _A_in["x"],
        "A_w_r": _A_in["w_r"],
        "A_w_i": _A_in["w_i"],
        "B_x": _B_in["x"],
        "B_wqkv": _B_in["wqkv"],
        "B_wo": _B_in["wo"],
    }

def reference(A_x, A_w_r, A_w_i, B_x, B_wqkv, B_wo):
    def _A_ref(x, w_r, w_i):
        B, S, D = x.shape
        X = (lambda x, axes=(-2,-1): jnp.fft.rfft2(x.astype(jnp.float32), axes=axes))(x, axes=(-2, -1))
        W = w_r + 1j * w_i
        X = X * W
        y = (lambda x, s, axes=(-2,-1): jnp.fft.irfft2(x, s=s, axes=axes).astype(jnp.bfloat16))(X, (S, D), axes=(-2, -1))
        return y

    def _B_ref(x, wqkv, wo):
        B, S, D = x.shape
        H = 32
        Dh = D // H
        qkv = (lambda x, *d: x.transpose(*d))((x @ wqkv).reshape(B, S, 3, H, Dh), 2, 0, 3, 1, 4)
        q, k, v = qkv[0], qkv[1], qkv[2]
        scores = jnp.einsum("bhqd,bhkd->bhqk", q, k) * (Dh ** -0.5)
        p = _softmax(scores, axis=-1)
        o = jnp.einsum("bhqk,bhkd->bhqd", p, v)
        return (lambda x, *d: x.transpose(*d))(o, 0, 2, 1, 3).reshape(B, S, D) @ wo

    a = _A_ref(A_x, A_w_r, A_w_i)
    b = _B_ref(B_x, B_wqkv, B_wo)
    return jnp.concatenate([a, b], axis=-1)
```

```python
import math

import jax
import jax.numpy as jnp
import numpy as np
import jax.experimental.pallas as pl
import jax.experimental.pallas.tpu as pltpu

S = 2048
D = 576
DF = D // 2 + 1
H = 32
DH = D // H
LP = 304
R1 = 16
R2 = 128
QB = 512
KC = 128
HPS = 128 // DH
NSLAB = -(-H // HPS)
F32 = jnp.float32
BF16 = jnp.bfloat16


def _dft_constants():
    l = np.arange(DF)
    d = np.arange(D)
    ph = 2.0 * np.pi * ((l[:, None] * d[None, :]) % D) / D
    fdt = np.zeros((2 * LP, D))
    fdt[:DF] = np.cos(ph)
    fdt[LP:LP + DF] = -np.sin(ph)
    c = np.where((l == 0) | (l == D // 2), 1.0, 2.0) / (S * D)
    gt = np.zeros((D, 2 * LP))
    gt[:, :DF] = (c[:, None] * np.cos(ph)).T
    gt[:, LP:LP + DF] = (-c[:, None] * np.sin(ph)).T
    n2 = np.arange(R2)
    mf = np.zeros((R1, 2 * R2, 2 * R2))
    for k1 in range(R1):
        p = 2.0 * np.pi * (((k1 + R1 * n2)[None, :] * n2[:, None]) % S) / S
        cc, ss = np.cos(p), np.sin(p)
        mf[k1] = np.block([[cc, -ss], [ss, cc]])
    b = lambda a: np.asarray(a.astype(np.float32), dtype=BF16)
    return b(fdt), b(gt), b(mf)


_FDT, _GT, _MF = _dft_constants()


def _radix4(a, sign):
    (r0, i0), (r1, i1), (r2, i2), (r3, i3) = a
    t0 = (r0 + r2, i0 + i2)
    t1 = (r0 - r2, i0 - i2)
    t2 = (r1 + r3, i1 + i3)
    t3 = (r1 - r3, i1 - i3)
    x0 = (t0[0] + t2[0], t0[1] + t2[1])
    x2 = (t0[0] - t2[0], t0[1] - t2[1])
    xa = (t1[0] + t3[1], t1[1] - t3[0])
    xb = (t1[0] - t3[1], t1[1] + t3[0])
    return [x0, xa, x2, xb] if sign < 0 else [x0, xb, x2, xa]


def _twiddle16(z, e, sign):
    e %= 16
    r, i = z
    if e == 0:
        return z
    if e == 4:
        return (i, -r) if sign < 0 else (-i, r)
    c = math.cos(2.0 * math.pi * e / 16)
    s = sign * math.sin(2.0 * math.pi * e / 16)
    if e % 4 == 2:
        if c * s > 0:
            return ((r - i) * c, (r + i) * c)
        return ((r + i) * c, (i - r) * c)
    return (r * c - i * s, r * s + i * c)


def _fft16(x, sign):
    t = [_radix4([x[4 * a + b] for a in range(4)], sign) for b in range(4)]
    out = [None] * 16
    for c in range(4):
        r = _radix4([_twiddle16(t[b][c], b * c, sign) for b in range(4)], sign)
        for d in range(4):
            out[c + 4 * d] = r[d]
    return out


def _nt(a, b):
    return jax.lax.dot_general(a, b, (((1,), (1,)), ((), ())), preferred_element_type=F32)


def _tn(a, b):
    return jax.lax.dot_general(a, b, (((0,), (0,)), ((), ())), preferred_element_type=F32)


def _tt(a, b):
    return jax.lax.dot_general(a, b, (((0,), (1,)), ((), ())), preferred_element_type=F32)


def _kernel(
    xa_h, wr_h, wi_h, xb_h, wqkv_h, wo_h, fdt_h, gt_h, mf_h,
    out_h,
    xa_v, wr_v, wi_v, xb_v, wqkv_v, wo_v, fdt_v, gt_v, mf_v,
    w32_v, xt_v, a_v, c_v, zt_v,
    k_v, qt_v, vt_v, vtc_v, s0_v, s1_v, m0_v, m1_v, ot_v, out_v,
    in_sem, out_sem,
):
    srcs = (xa_h, fdt_h, wr_h, wi_h, mf_h, gt_h, xb_h, wqkv_h, wo_h)
    dsts = (xa_v, fdt_v, wr_v, wi_v, mf_v, gt_v, xb_v, wqkv_v, wo_v)
    cps = [pltpu.make_async_copy(s_, d_, in_sem.at[n]) for n, (s_, d_) in enumerate(zip(srcs, dsts))]
    for cp in cps:
        cp.start()

    cps[0].wait()
    cps[1].wait()
    with jax.named_scope("A_dfwd"):
        xt_v[...] = jnp.dot(fdt_v[...], xa_v[...], preferred_element_type=F32)

    with jax.named_scope("A_fft1"):
        def fft_fwd(r, carry):
            r0 = pl.multiple_of(r * 16, 16)
            x = [(xt_v[pl.ds(r0, 16), n * R2:(n + 1) * R2],
                  xt_v[pl.ds(LP + r0, 16), n * R2:(n + 1) * R2]) for n in range(R1)]
            y = _fft16(x, -1)
            for k1 in range(R1):
                a_v[k1, pl.ds(r0, 16), 0:R2] = y[k1][0].astype(BF16)
                a_v[k1, pl.ds(r0, 16), R2:2 * R2] = y[k1][1].astype(BF16)
            return carry
        jax.lax.fori_loop(0, LP // 16, fft_fwd, 0)

    cps[2].wait()
    cps[3].wait()
    cps[4].wait()
    with jax.named_scope("A_wprep"):
        for n, w_v in enumerate((wr_v, wi_v)):
            for rc in range(S // 128):
                cols = slice(rc * 128, (rc + 1) * 128)
                w32_v[n, 0, cols, :] = w_v[0:128, cols].astype(F32).T
                w32_v[n, 1, cols, :] = w_v[128:256, cols].astype(F32).T
                tail = jnp.concatenate([w_v[256:DF, cols].astype(F32), jnp.zeros((384 - DF, 128), F32)], axis=0)
                w32_v[n, 2, cols, :] = tail.T

    with jax.named_scope("A_mid"):
        def mid(k1, carry):
            m = mf_v[k1]
            b = jnp.dot(a_v[k1], m, preferred_element_type=F32)
            for j in range(3):
                nr = min(128, LP - 128 * j)
                wr = w32_v[0, j, pl.ds(k1, R2, stride=R1), :].T[0:nr]
                wi = w32_v[1, j, pl.ds(k1, R2, stride=R1), :].T[0:nr]
                br = b[128 * j:128 * j + nr, 0:R2]
                bi = b[128 * j:128 * j + nr, R2:2 * R2]
                y = jnp.concatenate([br * wr - bi * wi, br * wi + bi * wr], axis=1).astype(BF16)
                c_v[k1, 128 * j:128 * j + nr, :] = _nt(y, m)
            return carry
        jax.lax.fori_loop(0, R1, mid, 0)

    with jax.named_scope("A_fft2"):
        def fft_inv(r, carry):
            r0 = pl.multiple_of(r * 16, 16)
            x = [(c_v[k1, pl.ds(r0, 16), 0:R2], c_v[k1, pl.ds(r0, 16), R2:2 * R2]) for k1 in range(R1)]
            y = _fft16(x, +1)
            for n in range(R1):
                zt_v[pl.ds(r0, 16), n * R2:(n + 1) * R2] = y[n][0].astype(BF16)
                zt_v[pl.ds(LP + r0, 16), n * R2:(n + 1) * R2] = y[n][1].astype(BF16)
            return carry
        jax.lax.fori_loop(0, LP // 16, fft_inv, 0)

    cps[5].wait()
    with jax.named_scope("A_dinv"):
        for sc in range(S // 512):
            yt = jnp.dot(gt_v[...], zt_v[:, sc * 512:(sc + 1) * 512], preferred_element_type=F32)
            out_v[sc * 512:(sc + 1) * 512, 0:D] = yt.T.astype(BF16)

    cps[6].wait()
    cps[7].wait()
    qscale = (DH ** -0.5) * math.log2(math.e)
    with jax.named_scope("B_qkv"):
        xb = xb_v[...]
        for s in range(NSLAB):
            c0 = HPS * DH * s
            qt_v[s] = (_tn(wqkv_v[:, c0:c0 + 128], xb) * qscale).astype(BF16)
            k_v[s] = _tn(wqkv_v[:, D + c0:D + c0 + 128], xb).T.astype(BF16)
        vtc_v[...] = _tn(wqkv_v[:, 2 * D:3 * D], xb)
        rows24 = jax.lax.broadcasted_iota(jnp.int32, (24, S), 0)
        ones8 = jnp.ones((8, S), F32)
        for h in range(H):
            w0 = (DH * h) // 8 * 8
            o = DH * h - w0
            v = jnp.where((rows24 >= o) & (rows24 < o + DH), vtc_v[w0:w0 + 24, :], 0.0)
            vt_v[h] = jnp.concatenate([v, ones8], axis=0).astype(BF16)
        ot_v[...] = jnp.zeros_like(ot_v)

    NT = (S // QB) * H
    NC = S // KC

    def stage(t1, t2, sw, mw, sr, mr):
        if t1 is not None:
            j1 = t1 // H
            h1 = t1 % H
            slab = h1 // HPS
            jj = h1 % HPS
            qt = qt_v[slab, :, pl.ds(pl.multiple_of(j1 * QB, QB), QB)]
            rows = jax.lax.broadcasted_iota(jnp.int32, (128, QB), 0)
            qm = jnp.where((rows >= DH * jj) & (rows < DH * jj + DH), qt, jnp.zeros_like(qt))
        if t2 is not None:
            j2 = t2 // H
            h2 = t2 % H
            mprev = mr[...]
        m = None
        acc = None
        for c in range(NC):
            ks = slice(c * KC, (c + 1) * KC)
            if t1 is not None:
                s = jnp.dot(k_v[slab, ks, :], qm, preferred_element_type=F32)
                sw[ks, :] = s
                mm = jnp.max(s.reshape(KC // 8, 8, QB), axis=0)
                m = mm if m is None else jnp.maximum(m, mm)
            if t2 is not None:
                s2 = sr[ks, :]
                p = jnp.exp2(s2.reshape(KC // 8, 8, QB) - mprev[None]).reshape(KC, QB).astype(BF16)
                a = jnp.dot(vt_v[h2, :, ks], p, preferred_element_type=F32)
                acc = a if acc is None else acc + a
        if t1 is not None:
            mw[...] = jnp.broadcast_to(jnp.max(m, axis=0, keepdims=True), (8, QB))
        if t2 is not None:
            o = acc[0:24].reshape(3, 8, QB) * (1.0 / acc[24:32])[None]
            w0 = pl.multiple_of((DH * h2) // 8 * 8, 8)
            qs = pl.ds(pl.multiple_of(j2 * QB, QB), QB)
            ot_v[pl.ds(w0, 24), qs] = ot_v[pl.ds(w0, 24), qs] + o.reshape(24, QB)

    cps[8].wait()

    def out_block(j):
        qs = pl.ds(pl.multiple_of(j * QB, QB), QB)
        ob = _tn(ot_v[:, qs].astype(BF16), wo_v[...])
        out_v[qs, D:2 * D] = ob.astype(BF16)

    def out_copy(j):
        qs = pl.ds(pl.multiple_of(j * QB, QB), QB)
        return pltpu.make_async_copy(out_v.at[qs], out_h.at[qs], out_sem.at[j])

    with jax.named_scope("B_attn"):
        stage(0, None, s0_v, m0_v, None, None)

        def body(u, carry):
            stage(2 * u + 1, 2 * u, s1_v, m1_v, s0_v, m0_v)
            stage(2 * u + 2, 2 * u + 1, s0_v, m0_v, s1_v, m1_v)

            @pl.when(u % (H // 2) == H // 2 - 1)
            def _():
                j = u // (H // 2)
                out_block(j)
                out_copy(j).start()
            return carry
        jax.lax.fori_loop(0, NT // 2 - 1, body, 0)
        stage(NT - 1, NT - 2, s1_v, m1_v, s0_v, m0_v)
        stage(None, NT - 1, None, None, s1_v, m1_v)
        out_block(S // QB - 1)
        out_copy(S // QB - 1).start()
    for j in range(S // QB):
        out_copy(j).wait()


@jax.jit
def pallas_concat_heads__spectral_gfnet__mha_block__prompt_kernel(
    A_x: jax.Array,
    A_w_r: jax.Array,
    A_w_i: jax.Array,
    B_x: jax.Array,
    B_wqkv: jax.Array,
    B_wo: jax.Array,
):
    assert A_x.shape == (1, S, D) and B_x.shape == (1, S, D)
    vm = pltpu.VMEM
    scratch = [
        vm((D, S), BF16), vm((DF, S), BF16), vm((DF, S), BF16), vm((D, S), BF16),
        vm((D, 3 * D), BF16), vm((D, D), BF16),
        vm((2 * LP, D), BF16), vm((D, 2 * LP), BF16), vm((R1, 2 * R2, 2 * R2), BF16),
        vm((2, 3, S, 128), F32),
        vm((2 * LP, S), F32),
        vm((R1, LP, 2 * R2), BF16),
        vm((R1, LP, 2 * R2), F32),
        vm((2 * LP, S), BF16),
        vm((NSLAB, S, 128), BF16),
        vm((NSLAB, 128, S), BF16),
        vm((H, 32, S), BF16),
        vm((D, S), F32),
        vm((S, QB), F32), vm((S, QB), F32), vm((8, QB), F32), vm((8, QB), F32),
        vm((D, S), F32),
        vm((S, 2 * D), BF16),
        pltpu.SemaphoreType.DMA((9,)),
        pltpu.SemaphoreType.DMA((S // QB,)),
    ]
    any_spec = pl.BlockSpec(memory_space=pltpu.HBM)
    out = pl.pallas_call(
        _kernel,
        out_shape=jax.ShapeDtypeStruct((S, 2 * D), BF16),
        in_specs=[any_spec] * 9,
        out_specs=any_spec,
        scratch_shapes=scratch,
        compiler_params=pltpu.CompilerParams(vmem_limit_bytes=110 * 1024 * 1024),
    )(
        A_x.reshape(S, D).T, A_w_r.T, A_w_i.T, B_x.reshape(S, D).T, B_wqkv, B_wo,
        _FDT, _GT, _MF,
    )
    return out.reshape(1, S, 2 * D)
```

```python
import functools
import math

import jax
import jax.numpy as jnp
import numpy as np
import jax.experimental.pallas as pl
import jax.experimental.pallas.tpu as pltpu

S = 2048
D = 576
DF = D // 2 + 1
H = 32
DH = D // H
NE = 152
NO = 144
LP = 304
R1 = 16
R2 = 128
QB = 512
KC = 128
HPS = 128 // DH
NSLAB = -(-H // HPS)
F32 = jnp.float32
BF16 = jnp.bfloat16


def _dft_constants():
    d = np.arange(D // 2)
    le = 2 * np.arange(D // 4 + 1)
    lo = 2 * np.arange(D // 4) + 1
    fwd, inv = [], []
    for l, n in ((le, NE), (lo, NO)):
        ph = 2.0 * np.pi * ((l[:, None] * d[None, :]) % D) / D
        f = np.zeros((2 * n, D // 2))
        f[:len(l)] = np.cos(ph)
        f[n:n + len(l)] = -np.sin(ph)
        c = np.where((l == 0) | (l == D // 2), 1.0, 2.0) / (S * D)
        fwd.append(f)
        inv.append((f.reshape(2, n, -1) * np.pad(c, (0, n - len(l)))[None, :, None]).reshape(2 * n, -1).T)
    fdt = np.concatenate(fwd, axis=0)
    gt = np.zeros((D, 2 * NE))
    gt[:D // 2] = inv[0]
    gt[D // 2:, :2 * NO] = inv[1]
    n2 = np.arange(R2)
    mf = np.zeros((R1, 2 * R2, 2 * R2))
    for k1 in range(R1):
        p = 2.0 * np.pi * (((k1 + R1 * n2)[None, :] * n2[:, None]) % S) / S
        cc, ss = np.cos(p), np.sin(p)
        mf[k1] = np.block([[cc, -ss], [ss, cc]])
    b = lambda a: np.asarray(a.astype(np.float32), dtype=BF16)
    return b(fdt), b(gt), b(mf)


_FDT, _GT, _MF = _dft_constants()


def _radix4(a, sign):
    (r0, i0), (r1, i1), (r2, i2), (r3, i3) = a
    t0 = (r0 + r2, i0 + i2)
    t1 = (r0 - r2, i0 - i2)
    t2 = (r1 + r3, i1 + i3)
    t3 = (r1 - r3, i1 - i3)
    x0 = (t0[0] + t2[0], t0[1] + t2[1])
    x2 = (t0[0] - t2[0], t0[1] - t2[1])
    xa = (t1[0] + t3[1], t1[1] - t3[0])
    xb = (t1[0] - t3[1], t1[1] + t3[0])
    return [x0, xa, x2, xb] if sign < 0 else [x0, xb, x2, xa]


def _twiddle16(z, e, sign):
    e %= 16
    r, i = z
    if e == 0:
        return z
    if e == 4:
        return (i, -r) if sign < 0 else (-i, r)
    c = math.cos(2.0 * math.pi * e / 16)
    s = sign * math.sin(2.0 * math.pi * e / 16)
    if e % 4 == 2:
        if c * s > 0:
            return ((r - i) * c, (r + i) * c)
        return ((r + i) * c, (i - r) * c)
    return (r * c - i * s, r * s + i * c)


def _fft16(x, sign):
    t = [_radix4([x[4 * a + b] for a in range(4)], sign) for b in range(4)]
    out = [None] * 16
    for c in range(4):
        r = _radix4([_twiddle16(t[b][c], b * c, sign) for b in range(4)], sign)
        for d in range(4):
            out[c + 4 * d] = r[d]
    return out


def _nt(a, b):
    return jax.lax.dot_general(a, b, (((1,), (1,)), ((), ())), preferred_element_type=F32)


def _tn(a, b):
    return jax.lax.dot_general(a, b, (((0,), (0,)), ((), ())), preferred_element_type=F32)


def _tt(a, b):
    return jax.lax.dot_general(a, b, (((0,), (1,)), ((), ())), preferred_element_type=F32)


def _kernel(
    xa_h, wr_h, wi_h, xb_h, wqkv_h, wo_h, fdt_h, gt_h, mf_h,
    out_h,
    xa_v, wr_v, wi_v, xb_v, wqkv_v, wo_v, fdt_v, gt_v, mf_v,
    w32_v, xt_v, a_v, c_v, zt_v,
    k_v, qt_v, vt_v, vtc_v, s0_v, s1_v, m0_v, m1_v, ot_v, out_v, wvt_v,
    in_sem, out_sem,
):
    NXA = 4
    XC = S // NXA
    cp_xa = [pltpu.make_async_copy(xa_h.at[:, c * XC:(c + 1) * XC], xa_v.at[:, c * XC:(c + 1) * XC], in_sem.at[c])
             for c in range(NXA)]
    names = ("fdt", "xb", "wqkv", "wr", "wi", "mf", "gt", "wo")
    srcs = (fdt_h, xb_h, wqkv_h, wr_h, wi_h, mf_h, gt_h, wo_h)
    dsts = (fdt_v, xb_v, wqkv_v, wr_v, wi_v, mf_v, gt_v, wo_v)
    cp = {n_: pltpu.make_async_copy(s_, d_, in_sem.at[NXA + i])
          for i, (n_, s_, d_) in enumerate(zip(names, srcs, dsts))}

    qscale = (DH ** -0.5) * math.log2(math.e)

    def dfwd(c):
        cs = slice(c * XC, (c + 1) * XC)
        lo_ = xa_v[0:D // 2, cs].astype(F32)
        hi_ = xa_v[D // 2:D, cs].astype(F32)
        e = jnp.dot(fdt_v[0:2 * NE, :], (lo_ + hi_).astype(BF16), preferred_element_type=F32)
        o = jnp.dot(fdt_v[2 * NE:, :], (lo_ - hi_).astype(BF16), preferred_element_type=F32)
        xt_v[0:NE, cs] = e[0:NE]
        xt_v[LP:LP + NE, cs] = e[NE:]
        xt_v[NE:NE + NO, cs] = o[0:NO]
        xt_v[LP + NE:LP + NE + NO, cs] = o[NO:]

    def fft_fwd(r):
        r0 = r * 8
        x = [(xt_v[r0:r0 + 8, n * R2:(n + 1) * R2],
              xt_v[LP + r0:LP + r0 + 8, n * R2:(n + 1) * R2]) for n in range(R1)]
        y = _fft16(x, -1)
        for k1 in range(R1):
            a_v[k1, r0:r0 + 8, 0:R2] = y[k1][0]
            a_v[k1, r0:r0 + 8, R2:2 * R2] = y[k1][1]

    def wprep(rc):
        cols = slice(rc * 128, (rc + 1) * 128)
        for n, w_v in enumerate((wr_v, wi_v)):
            pk = pltpu.bitcast(w_v[0:DF - 1, cols], jnp.uint32)
            ev = pltpu.bitcast(pk << 16, F32)
            od = pltpu.bitcast(pk & jnp.uint32(0xFFFF0000), F32)
            last = jnp.concatenate([w_v[DF - 1:DF, cols].astype(F32), jnp.zeros((7, 128), F32)], axis=0)
            w32_v[n, 0, cols, :] = ev[0:128].T
            w32_v[n, 1, cols, :] = jnp.concatenate([ev[128:], last, od[0:104]], axis=0).T
            w32_v[n, 2, cols, :] = jnp.concatenate([od[104:], jnp.zeros((88, 128), F32)], axis=0).T

    def mid1(k1):
        return jnp.dot(a_v[k1].astype(BF16), mf_v[k1], preferred_element_type=F32)

    def mid2(k1, b):
        ys = []
        for j in range(3):
            nr = min(128, LP - 128 * j)
            wr = w32_v[0, j, pl.ds(k1, R2, stride=R1), :].T[0:nr]
            wi = w32_v[1, j, pl.ds(k1, R2, stride=R1), :].T[0:nr]
            br = b[128 * j:128 * j + nr, 0:R2]
            bi = b[128 * j:128 * j + nr, R2:2 * R2]
            ys.append(jnp.concatenate([br * wr - bi * wi, br * wi + bi * wr], axis=1).astype(BF16))
        c_v[k1] = _nt(jnp.concatenate(ys, axis=0), mf_v[k1])

    def fft_inv(r):
        r0 = r * 8
        x = [(c_v[k1, r0:r0 + 8, 0:R2], c_v[k1, r0:r0 + 8, R2:2 * R2]) for k1 in range(R1)]
        y = _fft16(x, +1)
        for n in range(R1):
            zt_v[r0:r0 + 8, n * R2:(n + 1) * R2] = y[n][0]
            zt_v[LP + r0:LP + r0 + 8, n * R2:(n + 1) * R2] = y[n][1]

    def dinv(sc):
        cs = slice(sc * 256, (sc + 1) * 256)
        ze = jnp.concatenate([zt_v[0:NE, cs], zt_v[LP:LP + NE, cs]], axis=0).astype(BF16)
        zo = jnp.concatenate([zt_v[NE:NE + NO, cs], zt_v[LP + NE:LP + NE + NO, cs]], axis=0).astype(BF16)
        e = jnp.dot(gt_v[0:D // 2, :], ze, preferred_element_type=F32)
        o = jnp.dot(gt_v[D // 2:, 0:2 * NO], zo, preferred_element_type=F32)
        yt = jnp.concatenate([e + o, e - o], axis=0).astype(BF16)
        out_v[cs, 0:D] = yt.T

    def proj_q(s, c):
        cs = slice(c * XC, (c + 1) * XC)
        c0 = HPS * DH * s
        qt = (_tn(wqkv_v[:, c0:c0 + 128], xb_v[:, cs]) * qscale).astype(BF16)
        qt_v[s, :, cs] = qt

    def proj_k(s, c):
        cs = slice(c * XC, (c + 1) * XC)
        c0 = D + HPS * DH * s
        kt = _tn(wqkv_v[:, c0:c0 + 128], xb_v[:, cs]).astype(BF16)
        k_v[s, cs, :] = kt.T

    def proj_v(c, g):
        cs = slice(c * XC, (c + 1) * XC)
        rs = slice(g * 144, (g + 1) * 144)
        vtc_v[rs, cs] = jnp.dot(wvt_v[rs, :], xb_v[:, cs], preferred_element_type=F32)

    def v_layout(h):
        rows24 = jax.lax.broadcasted_iota(jnp.int32, (24, S), 0)
        w0 = (DH * h) // 8 * 8
        o = DH * h - w0
        v = jnp.where((rows24 >= o) & (rows24 < o + DH), vtc_v[w0:w0 + 24, :], 0.0)
        vt_v[h] = jnp.concatenate([v, jnp.ones((8, S), F32)], axis=0).astype(BF16)

    cp["fdt"].start()
    for c in range(NXA):
        cp_xa[c].start()
    cp["fdt"].wait()
    cp_xa[0].wait()
    dfwd(0)
    cp_xa[1].wait()
    cp["xb"].start()
    cp["wqkv"].start()
    dfwd(1)
    cp_xa[2].wait()
    dfwd(2)
    cp_xa[3].wait()
    dfwd(3)
    for r in range(16):
        fft_fwd(r)
    cp["xb"].wait()
    cp["wqkv"].wait()
    for n_ in ("wr", "wi", "mf", "gt", "wo"):
        cp[n_].start()
    ot_v[...] = jnp.zeros_like(ot_v)
    for k1 in range(R1):
        a_v[k1, 296:LP, :] = jnp.zeros((LP - 296, 2 * R2), F32)
    wvt_v[...] = wqkv_v[:, 2 * D:3 * D].T

    def interleave(mxu_tasks, vpu_tasks):
        n, m = len(mxu_tasks), len(vpu_tasks)
        for i, t in enumerate(mxu_tasks):
            for v in vpu_tasks[i * m // n:(i + 1) * m // n]:
                v()
            t()

    P = functools.partial
    nfft = 296 // 8
    interleave([P(proj_v, c, g) for c in range(NXA) for g in range(4)],
               [P(fft_fwd, r) for r in range(16, nfft)])
    cp["wr"].wait()
    cp["wi"].wait()
    kq = [(s_, c) for s_ in range(NSLAB) for c in range(NXA)]
    side = []
    for i in range(16):
        side += [P(wprep, i), P(v_layout, 2 * i), P(v_layout, 2 * i + 1)]
    interleave([P(proj_k, s_, c) for s_, c in kq], side)
    cp["mf"].wait()
    b = mid1(0)
    for k1 in range(R1):
        bn = mid1(k1 + 1) if k1 + 1 < R1 else None
        mid2(k1, b)
        b = bn
    proj_q(*kq[0])
    interleave([P(proj_q, s_, c) for s_, c in kq[1:]], [P(fft_inv, r) for r in range(nfft)])
    cp["gt"].wait()
    for i in range(S // 256):
        dinv(i)

    NC = S // KC
    NQ = S // QB

    def stage(u1, u2, sw, mw, sr, mr):
        if u1 is not None:
            h1, j1 = u1
            w1 = QB
            slab = h1 // HPS
            jj = h1 % HPS
            qt = qt_v[slab, :, j1 * QB:j1 * QB + w1]
            rows = jax.lax.broadcasted_iota(jnp.int32, (128, w1), 0)
            qm = jnp.where((rows >= DH * jj) & (rows < DH * jj + DH), qt, jnp.zeros_like(qt))
        if u2 is not None:
            h2, j2 = u2
            w2 = QB
            mprev = mr[:, 0:w2]
        m = None
        acc = None
        for c in range(NC):
            ks = slice(c * KC, (c + 1) * KC)
            if u1 is not None:
                s = jnp.dot(k_v[slab, ks, :], qm, preferred_element_type=F32)
                sw[ks, 0:w1] = s
                mm = jnp.max(s.reshape(KC // 8, 8, w1), axis=0)
                m = mm if m is None else jnp.maximum(m, mm)
            if u2 is not None:
                s2 = sr[ks, 0:w2]
                p = jnp.exp2(s2.reshape(KC // 8, 8, w2) - mprev[None]).reshape(KC, w2).astype(BF16)
                vt = vt_v[h2, :, ks]
                a = jnp.dot(vt, p, preferred_element_type=F32)
                acc = a if acc is None else acc + a
        if u1 is not None:
            mw[:, 0:w1] = jnp.broadcast_to(jnp.max(m, axis=0, keepdims=True), (8, w1))
        if u2 is not None:
            w0 = pl.multiple_of((DH * h2) // 8 * 8, 8)
            pieces = [(acc, j2 * QB, w2)]
            for ac, q0, w in pieces:
                o = ac[0:24].reshape(3, 8, w) * (1.0 / ac[24:32])[None]
                ot_v[pl.ds(w0, 24), q0:q0 + w] = ot_v[pl.ds(w0, 24), q0:q0 + w] + o.reshape(24, w)

    cp["wo"].wait()

    def out_block(j):
        qs = slice(j * QB, (j + 1) * QB)
        ob = _tn(ot_v[:, qs].astype(BF16), wo_v[...])
        out_v[qs, D:2 * D] = ob.astype(BF16)

    def out_copy(j):
        qs = slice(j * QB, (j + 1) * QB)
        return pltpu.make_async_copy(out_v.at[qs], out_h.at[qs], out_sem.at[j])

    def head(h, last):
        bufs = ((s0_v, m0_v), (s1_v, m1_v))
        for k in range(NQ):
            if k + 1 < NQ:
                u1 = (h, k + 1)
            else:
                u1 = None if last else (h + 1, 0)
            stage(u1, (h, k), *bufs[(k + 1) % 2], *bufs[k % 2])

    stage((0, 0), None, s0_v, m0_v, None, None)

    def body(h, carry):
        head(h, False)
        return carry
    jax.lax.fori_loop(0, H - 1, body, 0)
    head(H - 1, True)
    for j in range(NQ):
        out_block(j)
        out_copy(j).start()
    for j in range(S // QB):
        out_copy(j).wait()


@jax.jit
def pallas_concat_heads__spectral_gfnet__mha_block__prompt_kernel(
    A_x: jax.Array,
    A_w_r: jax.Array,
    A_w_i: jax.Array,
    B_x: jax.Array,
    B_wqkv: jax.Array,
    B_wo: jax.Array,
):
    assert A_x.shape == (1, S, D) and B_x.shape == (1, S, D)
    vm = pltpu.VMEM
    scratch = [
        vm((D, S), BF16), vm((DF, S), BF16), vm((DF, S), BF16), vm((D, S), BF16),
        vm((D, 3 * D), BF16), vm((D, D), BF16),
        vm((2 * NE + 2 * NO, D // 2), BF16), vm((D, 2 * NE), BF16), vm((R1, 2 * R2, 2 * R2), BF16),
        vm((2, 3, S, 128), F32),
        vm((2 * LP, S), F32),
        vm((R1, LP, 2 * R2), F32),
        vm((R1, LP, 2 * R2), F32),
        vm((2 * LP, S), F32),
        vm((NSLAB, S, 128), BF16),
        vm((NSLAB, 128, S), BF16),
        vm((H, 32, S), BF16),
        vm((D, S), F32),
        vm((S, QB), F32), vm((S, QB), F32), vm((8, QB), F32), vm((8, QB), F32),
        vm((D, S), F32),
        vm((S, 2 * D), BF16),
        vm((D, D), BF16),
        pltpu.SemaphoreType.DMA((12,)),
        pltpu.SemaphoreType.DMA((S // QB,)),
    ]
    any_spec = pl.BlockSpec(memory_space=pltpu.HBM)
    out = pl.pallas_call(
        _kernel,
        out_shape=jax.ShapeDtypeStruct((S, 2 * D), BF16),
        in_specs=[any_spec] * 9,
        out_specs=any_spec,
        scratch_shapes=scratch,
        compiler_params=pltpu.CompilerParams(vmem_limit_bytes=110 * 1024 * 1024),
    )(
        A_x.reshape(S, D).T, A_w_r.T, A_w_i.T, B_x.reshape(S, D).T, B_wqkv, B_wo,
        _FDT, _GT, _MF,
    )
    return out.reshape(1, S, 2 * D)
```
